```python
import os as _os
_os.environ.setdefault("JAX_PLATFORMS", "cpu")
import jax
import jax.numpy as jnp

def _softmax(x, axis=-1):
    return jax.nn.softmax(x, axis=axis)
def _gelu(x):
    return jax.nn.gelu(x, approximate=True)
def _silu(x):
    return jax.nn.silu(x)
def _sigmoid(x):
    return jax.nn.sigmoid(x)
def _layernorm(x, axis=-1, eps=1e-5):
    m = jnp.mean(x, axis=axis, keepdims=True)
    v = jnp.var(x, axis=axis, keepdims=True)
    return (x - m) / jnp.sqrt(v + eps)
def _scatter_add(tgt, idx, src, axis=0):
    return tgt.at[idx].add(src)
def _segment_sum(src, seg, n):
    return jax.ops.segment_sum(src, seg, n)
class _Rng:
    def __init__(self, key):
        self._k = key
    def _next(self):
        self._k, sub = jax.random.split(self._k)
        return sub
    def normal(self, shape):
        return jax.random.normal(self._next(), shape, dtype=jnp.bfloat16)
    def randint(self, lo, hi, shape):
        return jax.random.randint(self._next(), shape, lo, hi, dtype=jnp.int32)
    def uniform(self, shape, lo=0.0, hi=1.0):
        return jax.random.uniform(self._next(), shape, jnp.bfloat16, lo, hi)
    def permutation(self, n):
        return jax.random.permutation(self._next(), n)


kernel_name = 'sequential_preLN__softmax_full_mha__glu_gated_swiglu__prompt'

def setup_inputs():
    _rng = _Rng(jax.random.key(int.from_bytes(__import__("os").urandom(4), "little")))
    _w = (lambda a: (lambda t: t.astype(jnp.bfloat16) if jnp.issubdtype(t.dtype, jnp.floating) else t)(jnp.asarray(a)))
    def _A_setup():
        B, S, D = 1, 2048, 640
        return {
            "x": _w((lambda *s: _rng.normal(s) * 0.05)(B, S, D)),
            "wqkv": _w((lambda *s: _rng.normal(s) * 0.05)(D, 3 * D)),
            "wo": _w((lambda *s: _rng.normal(s) * 0.05)(D, D)),
        }
    _A_in = _A_setup()

    def _B_setup():
        B, S, D, F = 1, 2048, 640, 1728
        return {
            "x": _w((lambda *s: _rng.normal(s) * 0.05)(B, S, D)),
            "w1": _w((lambda *s: _rng.normal(s) * 0.05)(D, F) * (2.0 / D) ** 0.5),
            "w3": _w((lambda *s: _rng.normal(s) * 0.05)(D, F) * (2.0 / D) ** 0.5),
            "w2": _w((lambda *s: _rng.normal(s) * 0.05)(F, D) * (2.0 / F) ** 0.5),
        }
    _B_in = _B_setup()

    return {
        "A_x": _A_in["x"],
        "A_wqkv": _A_in["wqkv"],
        "A_wo": _A_in["wo"],
        "B_x": _B_in["x"],
        "B_w1": _B_in["w1"],
        "B_w3": _B_in["w3"],
        "B_w2": _B_in["w2"],
    }

def reference(A_x, A_wqkv, A_wo, B_x, B_w1, B_w3, B_w2):
    def _A_ref(x, wqkv, wo):
        B, S, D = x.shape
        H = 32; Dh = D // H
        qkv = (lambda x, *d: x.transpose(*d))((x @ wqkv).reshape(B, S, 3, H, Dh), 2, 0, 3, 1, 4)
        q, k, v = qkv[0], qkv[1], qkv[2]
        scale = Dh ** -0.5
        scores = jnp.einsum("bhqd,bhkd->bhqk", q, k) * scale
        p = _softmax(scores, axis=-1)
        o = jnp.einsum("bhqk,bhkd->bhqd", p, v)
        return (lambda x, *d: x.transpose(*d))(o, 0, 2, 1, 3).reshape(B, S, D) @ wo

    def _B_ref(x, w1, w3, w2):
        gate = jnp.einsum("bsd,df->bsf", x, w1)
        up = jnp.einsum("bsd,df->bsf", x, w3)
        h = _silu(gate) * up
        out = jnp.einsum("bsf,fd->bsd", h, w2)
        return out

    x = A_x
    h = x + _A_ref(_layernorm(x, axis=-1), A_wqkv, A_wo)
    h2 = h + _B_ref(_layernorm(h, axis=-1), B_w1, B_w3, B_w2)
    return h2
```

```python
import functools

import jax
import jax.numpy as jnp
from jax import lax
import jax.experimental.pallas as pl
import jax.experimental.pallas.tpu as pltpu

S = 2048
D = 640
H = 32
DH = D // H
DHP = 24
HP = H * DHP
F = 1728
EPS = 1e-5
SCALE = DH ** -0.5

TQ = 256
QKV_COL_CHUNK = 512


def _layernorm_cols(xT):
    m = jnp.mean(xT, axis=0, keepdims=True)
    c = xT - m
    v = jnp.mean(c * c, axis=0, keepdims=True)
    return c / jnp.sqrt(v + EPS)


def _kernel(xT_ref, wqkvT_ref, woT_ref, w1T_ref, w3T_ref, w2T_ref,
            out_ref,
            qkvT_scr, knat_scr, oT_scr):
    i = pl.program_id(0)

    @pl.when(i == 0)
    def _prologue():
        for j in range(S // QKV_COL_CHUNK):
            cols = pl.ds(j * QKV_COL_CHUNK, QKV_COL_CHUNK)
            xT = xT_ref[:, cols].astype(jnp.float32)
            xnT = _layernorm_cols(xT).astype(jnp.bfloat16)
            qkvT = jnp.dot(wqkvT_ref[...], xnT, preferred_element_type=jnp.float32)
            qkvT_scr[0:HP, cols] = qkvT[0:HP, :] * SCALE
            qkvT_scr[HP:3 * HP, cols] = qkvT[HP:3 * HP, :]
        for h in range(H):
            qkvT_scr[pl.ds(2 * HP + h * DHP + DH, 1), :] = jnp.ones((1, S), jnp.float32)
            knat_scr[h] = qkvT_scr[pl.ds(HP + h * DHP, DHP), :].T.astype(jnp.bfloat16)

    qcols = pl.ds(pl.multiple_of(i * TQ, TQ), TQ)

    def head_body(h, carry):
        r = pl.multiple_of(h * DHP, 8)
        qT = qkvT_scr[pl.ds(r, DHP), qcols].astype(jnp.bfloat16)
        vT = qkvT_scr[pl.ds(2 * HP + r, DHP), :].astype(jnp.bfloat16)
        sT = jnp.dot(knat_scr[h], qT, preferred_element_type=jnp.float32)
        mT = jnp.max(sT, axis=0, keepdims=True)
        pT = jnp.exp(sT - mT).astype(jnp.bfloat16)
        oT = jnp.dot(vT, pT, preferred_element_type=jnp.float32)
        oT_scr[pl.ds(r, DHP), :] = oT / oT[DH:DH + 1, :]
        return carry

    lax.fori_loop(0, H, head_body, 0)

    xT = xT_ref[:, qcols].astype(jnp.float32)
    oallT = oT_scr[...].astype(jnp.bfloat16)
    attnT = jnp.dot(woT_ref[...], oallT, preferred_element_type=jnp.float32)
    hT = xT + attnT

    hnT = _layernorm_cols(hT).astype(jnp.bfloat16)
    gateT = jnp.dot(w1T_ref[...], hnT, preferred_element_type=jnp.float32)
    upT = jnp.dot(w3T_ref[...], hnT, preferred_element_type=jnp.float32)
    hmidT = (gateT * jax.nn.sigmoid(gateT) * upT).astype(jnp.bfloat16)
    ffnT = jnp.dot(w2T_ref[...], hmidT, preferred_element_type=jnp.float32)
    outT = hT + ffnT
    out_ref[...] = outT.T.astype(out_ref.dtype)


@jax.jit
def pallas_sequential_preLN__softmax_full_mha__glu_gated_swiglu__prompt_kernel(
    A_x: jax.Array,
    A_wqkv: jax.Array,
    A_wo: jax.Array,
    B_x: jax.Array,
    B_w1: jax.Array,
    B_w3: jax.Array,
    B_w2: jax.Array,
):
    del B_x
    xT = A_x.reshape(S, D).T
    wqkvT = jnp.pad(A_wqkv.reshape(D, 3, H, DH),
                    ((0, 0), (0, 0), (0, 0), (0, DHP - DH))).reshape(D, 3 * HP).T
    woT = jnp.pad(A_wo.reshape(H, DH, D),
                  ((0, 0), (0, DHP - DH), (0, 0))).reshape(HP, D).T
    w1T = B_w1.T
    w3T = B_w3.T
    w2T = B_w2.T

    grid = (S // TQ,)
    out = pl.pallas_call(
        _kernel,
        grid=grid,
        in_specs=[
            pl.BlockSpec((D, S), lambda i: (0, 0)),
            pl.BlockSpec((3 * HP, D), lambda i: (0, 0)),
            pl.BlockSpec((D, HP), lambda i: (0, 0)),
            pl.BlockSpec((F, D), lambda i: (0, 0)),
            pl.BlockSpec((F, D), lambda i: (0, 0)),
            pl.BlockSpec((D, F), lambda i: (0, 0)),
        ],
        out_specs=pl.BlockSpec((TQ, D), lambda i: (i, 0)),
        out_shape=jax.ShapeDtypeStruct((S, D), jnp.bfloat16),
        scratch_shapes=[
            pltpu.VMEM((3 * HP, S), jnp.float32),
            pltpu.VMEM((H, S, DHP), jnp.bfloat16),
            pltpu.VMEM((HP, TQ), jnp.float32),
        ],
        compiler_params=pltpu.CompilerParams(
            dimension_semantics=("arbitrary",),
            vmem_limit_bytes=110 * 1024 * 1024,
        ),
    )(xT, wqkvT, woT, w1T, w3T, w2T)
    return out.reshape(1, S, D)
```
